```python
import os as _os
_os.environ.setdefault("JAX_PLATFORMS", "cpu")
import jax
import jax.numpy as jnp

def _softmax(x, axis=-1):
    return jax.nn.softmax(x, axis=axis)
def _gelu(x):
    return jax.nn.gelu(x, approximate=True)
def _silu(x):
    return jax.nn.silu(x)
def _sigmoid(x):
    return jax.nn.sigmoid(x)
def _layernorm(x, axis=-1, eps=1e-5):
    m = jnp.mean(x, axis=axis, keepdims=True)
    v = jnp.var(x, axis=axis, keepdims=True)
    return (x - m) / jnp.sqrt(v + eps)
def _scatter_add(tgt, idx, src, axis=0):
    return tgt.at[idx].add(src)
def _segment_sum(src, seg, n):
    return jax.ops.segment_sum(src, seg, n)
class _Rng:
    def __init__(self, key):
        self._k = key
    def _next(self):
        self._k, sub = jax.random.split(self._k)
        return sub
    def normal(self, shape):
        return jax.random.normal(self._next(), shape, dtype=jnp.bfloat16)
    def randint(self, lo, hi, shape):
        return jax.random.randint(self._next(), shape, lo, hi, dtype=jnp.int32)
    def uniform(self, shape, lo=0.0, hi=1.0):
        return jax.random.uniform(self._next(), shape, jnp.bfloat16, lo, hi)
    def permutation(self, n):
        return jax.random.permutation(self._next(), n)


kernel_name = 'standalone__gqa_block_cached__sampling'

def setup_inputs():
    _rng = _Rng(jax.random.key(int.from_bytes(__import__("os").urandom(4), "little")))
    _w = (lambda a: (lambda t: t.astype(jnp.bfloat16) if jnp.issubdtype(t.dtype, jnp.floating) else t)(jnp.asarray(a)))
    B, Sq, D = 32, 16, 1024
    Hq, Hkv, Sk, Dh = 32, 4, 2048, 128
    assert Hq % Hkv == 0, (Hq, Hkv)
    return {
        "x": _w((lambda *s: _rng.normal(s) * 0.8)(B, Sq, D)),
        "k_cache": _w((lambda *s: _rng.normal(s) * 0.8)(B, Hkv, Sk, Dh)),
        "v_cache": _w((lambda *s: _rng.normal(s) * 0.05)(B, Hkv, Sk, Dh)),
        "wq": _w((lambda *s: _rng.normal(s) * 0.8)(D, Hq * Dh) * (D ** -0.5)),
        "wo": _w((lambda *s: _rng.normal(s) * 0.05)(Hq * Dh, D) * ((Hq * Dh) ** -0.5)),
    }

def reference(x, k_cache, v_cache, wq, wo):
    B, Sq, D = x.shape
    Hq, Dh = 32, 128
    Hkv = k_cache.shape[1]
    rep = Hq // Hkv
    q = (lambda x, *d: x.transpose(*d))((x @ wq).reshape(B, Sq, Hq, Dh), 0, 2, 1, 3)
    k = jnp.repeat(k_cache, rep, axis=1)
    v = jnp.repeat(v_cache, rep, axis=1)
    scores = jnp.einsum("bhqd,bhkd->bhqk", q, k) * (Dh ** -0.5)
    p = _softmax(scores, axis=-1)
    o = jnp.einsum("bhqk,bhkd->bhqd", p, v)
    return (lambda x, *d: x.transpose(*d))(o, 0, 2, 1, 3).reshape(B, Sq, Hq * Dh) @ wo
```

```python
import functools
import jax
import jax.numpy as jnp
import numpy as np
from jax import lax
from jax.experimental import pallas as pl
from jax.experimental.pallas import tpu as pltpu

NT = (((1,), (1,)), ((), ()))
LOG2E = 1.4426950408889634


def make(NB=8, prio=False, unroll=1):
    def kernel(x_hbm, k_hbm, v_hbm, wq_hbm, wo_hbm, out_hbm,
               x_v, wq_v, wo_v, kb, vb, q_s, o_s, acc, out_v,
               sem_kv, sem_x, sem_w, sem_o, *, B, Hkv, rep, Sq, Dh, G):
        ngrp = B // G
        npair = Hkv * B
        W = rep * Dh
        qscale = np.float32((Dh ** -0.5) * LOG2E)

        def kv_copy(i, slot):
            h = i // B
            b = i % B
            return (pltpu.make_async_copy(k_hbm.at[b, h], kb.at[slot], sem_kv.at[0, slot]),
                    pltpu.make_async_copy(v_hbm.at[b, h], vb.at[slot], sem_kv.at[1, slot]))

        def kv_start(i, slot):
            a, b = kv_copy(i, slot)
            if prio:
                a.start(priority=0); b.start(priority=1)
            else:
                a.start(); b.start()

        def wq_copy(h):
            return pltpu.make_async_copy(wq_hbm.at[:, pl.ds(h * W, W)], wq_v.at[h], sem_w.at[0, h])

        def wo_copy(h):
            return pltpu.make_async_copy(wo_hbm.at[pl.ds(h * W, W), :], wo_v.at[h], sem_w.at[1, h])

        x_copy = pltpu.make_async_copy(x_hbm, x_v, sem_x.at[0])
        x_copy.start()
        wq_copy(0).start()
        for i in range(NB):
            kv_start(i, i)
        wo_copy(0).start()
        for h in range(1, Hkv):
            wq_copy(h).start()
            wo_copy(h).start()
        x_copy.wait()

        def q_proj(h, g):
            xg = x_v[pl.ds(pl.multiple_of(g * (G * Sq), G * Sq), G * Sq), :]
            q = jnp.dot(xg, wq_v[h], preferred_element_type=jnp.float32) * qscale
            q = q.astype(jnp.bfloat16)
            for bl in range(G):
                for r in range(rep):
                    q_s[bl, r * Sq:(r + 1) * Sq, :] = q[bl * Sq:(bl + 1) * Sq, r * Dh:(r + 1) * Dh]

        def o_proj(h, g):
            y = jnp.dot(o_s[...], wo_v[h], preferred_element_type=jnp.float32)

            @pl.when(h == 0)
            def _():
                acc[g] = y

            @pl.when(jnp.logical_and(h > 0, h < Hkv - 1))
            def _():
                acc[g] += y

            @pl.when(h == Hkv - 1)
            def _():
                out_v[g] = (acc[g] + y).astype(out_v.dtype)
                pltpu.make_async_copy(out_v.at[g], out_hbm.at[pl.ds(pl.multiple_of(g * (G * Sq), G * Sq), G * Sq), :], sem_o.at[g]).start()

        def attend(i, bl, slot):
            q = q_s[bl]
            s = lax.dot_general(q, kb[slot], NT, preferred_element_type=jnp.float32)
            m = jnp.max(s, axis=-1, keepdims=True)
            p = jnp.exp2(s - m)
            l = jnp.sum(p, axis=-1, keepdims=True)
            o = jnp.dot(p.astype(jnp.bfloat16), vb[slot], preferred_element_type=jnp.float32)
            o = (o * (1.0 / l)).astype(jnp.bfloat16)
            for r in range(rep):
                o_s[pl.ds(pl.multiple_of(bl * Sq, Sq), Sq), r * Dh:(r + 1) * Dh] = o[r * Sq:(r + 1) * Sq, :]

        def unit(u, c):
            h = u // ngrp
            g = u % ngrp

            @pl.when(g == 0)
            def _():
                wq_copy(h).wait()
            q_proj(h, g)

            def pair(bl, c2):
                i = u * G + bl
                slot = i % NB
                a, b = kv_copy(i, slot)
                a.wait(); b.wait()
                attend(i, bl, slot)

                @pl.when(i + NB < npair)
                def _():
                    kv_start(i + NB, slot)
                return c2
            lax.fori_loop(0, G, pair, 0, unroll=unroll)

            @pl.when(g == 0)
            def _():
                wo_copy(h).wait()
            o_proj(h, g)
            return c
        lax.fori_loop(0, Hkv * ngrp, unit, 0)
        for g in range(ngrp):
            pltpu.make_async_copy(out_v.at[g], out_hbm.at[pl.ds(g * G * Sq, G * Sq), :], sem_o.at[g]).wait()

    def fn(x, k_cache, v_cache, wq, wo):
        B, Sq, D = x.shape
        _, Hkv, Sk, Dh = k_cache.shape
        Hq = wq.shape[1] // Dh
        rep = Hq // Hkv
        G = 8
        W = rep * Dh
        kern = functools.partial(kernel, B=B, Hkv=Hkv, rep=rep, Sq=Sq, Dh=Dh, G=G)
        bf = jnp.bfloat16
        out = pl.pallas_call(
            kern,
            out_shape=jax.ShapeDtypeStruct((B * Sq, D), x.dtype),
            in_specs=[pl.BlockSpec(memory_space=pl.ANY)] * 5,
            out_specs=pl.BlockSpec(memory_space=pl.ANY),
            scratch_shapes=[
                pltpu.VMEM((B * Sq, D), bf),
                pltpu.VMEM((Hkv, D, W), bf),
                pltpu.VMEM((Hkv, W, D), bf),
                pltpu.VMEM((NB, Sk, Dh), bf),
                pltpu.VMEM((NB, Sk, Dh), bf),
                pltpu.VMEM((G, rep * Sq, Dh), bf),
                pltpu.VMEM((G * Sq, W), bf),
                pltpu.VMEM((B // G, G * Sq, D), jnp.float32),
                pltpu.VMEM((B // G, G * Sq, D), bf),
                pltpu.SemaphoreType.DMA((2, NB)),
                pltpu.SemaphoreType.DMA((1,)),
                pltpu.SemaphoreType.DMA((2, Hkv)),
                pltpu.SemaphoreType.DMA((B // G,)),
            ],
            compiler_params=pltpu.CompilerParams(vmem_limit_bytes=100 << 20),
        )(x.reshape(B * Sq, D), k_cache, v_cache, wq, wo)
        return out.reshape(B, Sq, D)
    return fn


_impl = make(**dict(NB=4))


@jax.jit
def pallas_standalone__gqa_block_cached__sampling_kernel(
    x: jax.Array,
    k_cache: jax.Array,
    v_cache: jax.Array,
    wq: jax.Array,
    wo: jax.Array,
):
    return _impl(x, k_cache, v_cache, wq, wo)
```

```python
import functools
import jax
import jax.numpy as jnp
import numpy as np
from jax import lax
from jax.experimental import pallas as pl
from jax.experimental.pallas import tpu as pltpu

NT = (((1,), (1,)), ((), ()))
LOG2E = 1.4426950408889634


def make(NB=8, sub=128, pat='011', order='kkvv', wsub=16, wpat='011', nochk=True, nodma=False, nocomp=False,
         vwait='top', unroll=1, flags=None, osplit=1, prog='qom', mode='same', tile=128, delay=0):
    G = 8

    def kernel(x_hbm, k_hbm, v_hbm, wq_hbm, wo_hbm, out_hbm,
               kb, vb, x_v, wq_v, wo_v, q_s, o_s, acc, out_v, sem_kv, sem_x, sem_w, sem_o,
               *, B, Hkv, rep, Sq, Dh, Sk, D):
        ngrp = B // G
        nunit = Hkv * ngrp
        npair = nunit * G
        W = rep * Dh
        M = G * Sq
        qscale = np.float32((Dh ** -0.5) * LOG2E)
        ns = Sk // sub
        assert rep == G and W == D and NB <= G

        def kv_start(i, slot, order_=None):
            if nodma: return
            od = order_ or order
            u = i // G
            h = u // ngrp
            b = (u % ngrp) * G + i % G
            if od == 'kv': seq = [(a, j) for j in range(ns) for a in range(2)]
            elif od == 'KV': seq = [(a, j) for a in range(2) for j in range(ns)]
            elif od == 'kkvv': seq = [(a, j * 2 + t) for j in range(ns // 2) for a in range(2) for t in range(2)] if ns >= 2 else [(0, 0), (1, 0)]
            for c, (a, j) in enumerate(seq):
                src, dst = ((k_hbm, kb), (v_hbm, vb))[a]
                pltpu.make_async_copy(src.at[b, h, pl.ds(j * sub, sub)], dst.at[slot, pl.ds(j * sub, sub)],
                                      sem_kv.at[a, slot]).start(priority=int(pat[c % len(pat)]))

        def one(a, i, slot, j, prio):
            if nodma: return
            u = i // G
            h = u // ngrp
            b = (u % ngrp) * G + i % G
            src, dst = ((k_hbm, kb), (v_hbm, vb))[a]
            pltpu.make_async_copy(src.at[b, h, pl.ds(j * sub, sub)], dst.at[slot, pl.ds(j * sub, sub)],
                                  sem_kv.at[a, slot]).start(priority=prio)

        def kv_wait(a, slot):
            if nodma: return
            dst = (kb, vb)[a].at[slot]
            pltpu.make_async_copy(dst, dst, sem_kv.at[a, slot]).wait()

        def w_start(which, h, r0, nrows):
            if nodma: return
            for p in range(nrows // wsub):
                rr = r0 + p * wsub
                if not isinstance(rr, int):
                    rr = pl.multiple_of(rr, wsub)
                if which == 0:
                    hw = h * W
                    if not isinstance(hw, int):
                        hw = pl.multiple_of(hw, W)
                    src = wq_hbm.at[pl.ds(rr, wsub), pl.ds(hw, W)]
                    dst = wq_v.at[h, pl.ds(rr, wsub), :]
                else:
                    ro = h * W + rr
                    if not isinstance(ro, int):
                        ro = pl.multiple_of(ro, wsub)
                    src = wo_hbm.at[pl.ds(ro, wsub), :]
                    dst = wo_v.at[h, pl.ds(rr, wsub), :]
                pltpu.make_async_copy(src, dst, sem_w.at[which, h]).start(priority=int(wpat[p % len(wpat)]))

        def w_wait(which, h):
            if nodma: return
            dst = (wq_v, wo_v)[which].at[h]
            pltpu.make_async_copy(dst, dst, sem_w.at[which, h]).wait()

        def q_piece(u, r):
            h = u // ngrp
            g = u % ngrp
            xg = x_v[pl.ds(pl.multiple_of(g * M, M), M), :]
            w = wq_v[h, :, pl.ds(pl.multiple_of(r * Dh, Dh), Dh)]
            q = (jnp.dot(xg, w, preferred_element_type=jnp.float32) * qscale).astype(jnp.bfloat16)
            ro = pl.multiple_of(r * Sq, Sq)
            for bl in range(G):
                q_s[u % 2, bl, pl.ds(ro, Sq), :] = q[bl * Sq:(bl + 1) * Sq, :]

        def o_piece(u, n, width=None):
            width = width or Dh
            h = u // ngrp
            g = u % ngrp
            cs = pl.ds(pl.multiple_of(n * width, width), width) if not isinstance(n, int) else pl.ds(n * width, width)
            y = jnp.dot(o_s[u % 2], wo_v[h, :, cs], preferred_element_type=jnp.float32)
            t = acc[g, :, cs] + y
            acc[g, :, cs] = t
            out_v[g, :, cs] = t.astype(out_v.dtype)

        def out_start(g):
            gm = g * M if isinstance(g, int) else pl.multiple_of(g * M, M)
            return pltpu.make_async_copy(out_v.at[g], out_hbm.at[pl.ds(gm, M), :], sem_o.at[g])

        def body(i, c, do_q, do_o, phase):
            u = i // G
            bl = i % G
            h = u // ngrp
            g = u % ngrp
            slot = i % NB
            kv_wait(0, slot)
            if vwait == 'top':
                kv_wait(1, slot)
            nt = Sk // tile
            per = ns // nt
            pts = [[] for _ in range(2 * nt)]
            if mode == 'same':
                for t in range(nt):
                    for e in range(per):
                        pts[t].append((0, 0, t * per + e))
                        pts[nt + t].append((1, 0, t * per + e))
            elif mode == 'mix':
                kq = [(0, 0, j) for j in range(ns)]
                vq = [(1, -1, j) for j in range(ns // 2, ns)] + [(1, 0, j) for j in range(ns // 2)]
                for t in range(2 * nt):
                    for e in range(per):
                        c_ = t * per + e
                        pts[t].append(kq.pop(0) if c_ % 2 == 0 else vq.pop(0))
            cnt = [0]

            def issue(pt):
                for (a, off, j) in pts[pt]:
                    prio = int(pat[cnt[0] % len(pat)]); cnt[0] += 1
                    tgt = i + NB + off
                    if phase == 'C':
                        if npair - G + NB + off >= npair:
                            continue
                        @pl.when(tgt < npair)
                        def _():
                            one(a, tgt, tgt % NB, j, prio)
                        continue
                    if phase == 'A' and off == -1:
                        @pl.when(i > 0)
                        def _():
                            one(a, tgt, tgt % NB, j, prio)
                        continue
                    one(a, tgt, tgt % NB, j, prio)
            if phase == 'A':
                w_start(1, 0, bl * (W // G), W // G)
            elif phase == 'B':
                hs = W // 2
                pr = hs // G

                @pl.when(jnp.logical_and(g == 0, h > 0))
                def _():
                    w_start(1, h, hs + bl * pr, pr)

                @pl.when(jnp.logical_and(g == 1, h + 1 < Hkv))
                def _():
                    w_start(0, h + 1, bl * pr, pr)

                @pl.when(jnp.logical_and(g == 2, h + 1 < Hkv))
                def _():
                    w_start(0, h + 1, hs + bl * pr, pr)

                @pl.when(jnp.logical_and(g == 3, h + 1 < Hkv))
                def _():
                    w_start(1, h + 1, bl * pr, pr)

                @pl.when(jnp.logical_and(bl == 0, g == 1))
                def _():
                    w_wait(1, h)

                @pl.when(jnp.logical_and(bl == 0, jnp.logical_and(g == 3, h + 1 < Hkv)))
                def _():
                    w_wait(0, h + 1)
            if not nocomp:
                q = q_s[u % 2, bl]
                ss = []
                for t in range(nt):
                    kt = kb[slot, t * tile:(t + 1) * tile, :]
                    ss.append(lax.dot_general(q, kt, NT, preferred_element_type=jnp.float32))
                    issue(t)
                mm = ss[0]
                for t in range(1, nt):
                    mm = jnp.maximum(mm, ss[t])
                m = jnp.max(mm, axis=-1, keepdims=True)
                if prog == 'qom':
                    if do_q: q_piece(u + 1, bl)
                    if do_o: o_piece(u - 1, bl)
                if vwait == 'mid':
                    kv_wait(1, slot)
                o = None
                ll = None
                for t in range(nt):
                    p = jnp.exp2(ss[t] - m)
                    ll = p if ll is None else ll + p
                    pv = jnp.dot(p.astype(jnp.bfloat16), vb[slot, t * tile:(t + 1) * tile, :], preferred_element_type=jnp.float32)
                    o = pv if o is None else o + pv
                    issue(nt + t)
                l = jnp.sum(ll, axis=-1, keepdims=True)
                inv = pl.reciprocal(l, approx=True)
                inv = inv * (2.0 - l * inv)
                o = (o * inv).astype(jnp.bfloat16)
                if prog == 'mqo':
                    if do_q: q_piece(u + 1, bl)
                    if do_o: o_piece(u - 1, bl)
                ro = pl.multiple_of(bl * Sq, Sq)
                for r in range(rep):
                    o_s[u % 2, pl.ds(ro, Sq), r * Dh:(r + 1) * Dh] = o[r * Sq:(r + 1) * Sq, :]
            else:
                if vwait == 'mid':
                    kv_wait(1, slot)
                for t in range(2 * nt):
                    if delay: pl.delay(delay)
                    issue(t)
            if do_o:
                @pl.when(jnp.logical_and(bl == G - 1, u - 1 >= nunit - ngrp))
                def _():
                    out_start((u - 1) % ngrp).start()
            return c

        if not nodma:
            def pro(i, c):
                @pl.when(i == 0)
                def _():
                    pltpu.make_async_copy(x_hbm, x_v, sem_x.at[0]).start()
                    w_start(0, 0, 0, W)
                return c
            lax.fori_loop(0, 2, pro, 0)

            def pro2(i, c):
                kv_start(i, i)
                return c
            lax.fori_loop(0, NB, pro2, 0)
        acc[...] = jnp.zeros(acc.shape, acc.dtype)
        if not nodma:
            pltpu.make_async_copy(x_hbm, x_v, sem_x.at[0]).wait()
        w_wait(0, 0)
        if not nocomp:
            def pq(r, c):
                q_piece(0, r)
                return c
            lax.fori_loop(0, rep, pq, 0)

        lax.fori_loop(0, G, functools.partial(body, do_q=True, do_o=False, phase='A'), 0)
        lax.fori_loop(G, npair - G, functools.partial(body, do_q=True, do_o=True, phase='B'), 0, unroll=unroll)
        lax.fori_loop(npair - G, npair, functools.partial(body, do_q=False, do_o=True, phase='C'), 0)
        if not nocomp:
            wd = D // osplit
            for n in range(osplit):
                o_piece(nunit - 1, n, wd)
        out_start(ngrp - 1).start()
        for g in range(ngrp):
            out_start(g).wait()

    def fn(x, k_cache, v_cache, wq, wo):
        B, Sq, D = x.shape
        _, Hkv, Sk, Dh = k_cache.shape
        Hq = wq.shape[1] // Dh
        rep = Hq // Hkv
        W = rep * Dh
        kern = functools.partial(kernel, B=B, Hkv=Hkv, rep=rep, Sq=Sq, Dh=Dh, Sk=Sk, D=D)
        bf = jnp.bfloat16
        out = pl.pallas_call(
            kern,
            out_shape=jax.ShapeDtypeStruct((B * Sq, D), x.dtype),
            in_specs=[pl.BlockSpec(memory_space=pl.ANY)] * 5,
            out_specs=pl.BlockSpec(memory_space=pl.ANY),
            scratch_shapes=[
                pltpu.VMEM((NB, Sk, Dh), bf),
                pltpu.VMEM((NB, Sk, Dh), bf),
                pltpu.VMEM((B * Sq, D), bf),
                pltpu.VMEM((Hkv, D, W), bf),
                pltpu.VMEM((Hkv, W, D), bf),
                pltpu.VMEM((2, G, rep * Sq, Dh), bf),
                pltpu.VMEM((2, G * Sq, W), bf),
                pltpu.VMEM((B // G, G * Sq, D), jnp.float32),
                pltpu.VMEM((B // G, G * Sq, D), bf),
                pltpu.SemaphoreType.DMA((2, NB)),
                pltpu.SemaphoreType.DMA((1,)),
                pltpu.SemaphoreType.DMA((2, Hkv)),
                pltpu.SemaphoreType.DMA((B // G,)),
            ],
            compiler_params=pltpu.CompilerParams(vmem_limit_bytes=100 << 20, disable_bounds_checks=nochk, flags=flags),
        )(x.reshape(B * Sq, D), k_cache, v_cache, wq, wo)
        return out.reshape(B, Sq, D)
    return fn


_impl = make(**dict(mode='mix',NB=4))


@jax.jit
def pallas_standalone__gqa_block_cached__sampling_kernel(
    x: jax.Array,
    k_cache: jax.Array,
    v_cache: jax.Array,
    wq: jax.Array,
    wo: jax.Array,
):
    return _impl(x, k_cache, v_cache, wq, wo)
```

```python
import functools
import jax
import jax.numpy as jnp
import numpy as np
from jax import lax
from jax.experimental import pallas as pl
from jax.experimental.pallas import tpu as pltpu

NT = (((1,), (1,)), ((), ()))
LOG2E = 1.4426950408889634


def _shr(a, n):
    return a >> n if isinstance(a, int) else lax.shift_right_logical(a, jnp.int32(n))


def _mo(v, m):
    return v if isinstance(v, int) else pl.multiple_of(v, m)


def make(pat='011', wsub=64, wpat='0', wpos=15, nochk=True, nodma=False, nocomp=False, flags=None, unroll=1,
         msplit=True, dmid=True, xsub=512, xpat='0', ppat=None, lastsame=False, osplit=1, noepi=False, w0sub=None, w0pat=None, scopes=False, extra=None, kvpat='kv', pcont=False):
    import contextlib
    def sc(name):
        return jax.named_scope(name) if scopes else contextlib.nullcontext()
    G = 8
    NB = 4
    sub = 128
    ppat = ppat or pat
    w0sub_ = w0sub or wsub
    w0pat_ = w0pat or wpat

    def kernel(x_hbm, k_hbm, v_hbm, wq_hbm, wo_hbm, out_hbm,
               kb, vb, x_v, wq_v, wo_v, q_s, o_s, acc, out_v, sem_kv, sem_x, sem_w, sem_o,
               *, B, Hkv, rep, Sq, Dh, Sk, D):
        ngrp = B // G
        nunit = Hkv * ngrp
        npair = nunit * G
        W = rep * Dh
        M = G * Sq
        qscale = np.float32((Dh ** -0.5) * LOG2E)
        nt = Sk // sub
        assert rep == G and W == D and ngrp == 4 and Hkv == 4 and B == 32

        def one(a, i, j, prio):
            if nodma: return
            b, h = i & (B - 1), _shr(i, 5)
            slot = i & (NB - 1)
            src, dst = ((k_hbm, kb), (v_hbm, vb))[a]
            pltpu.make_async_copy(src.at[b, h, pl.ds(j * sub, sub)], dst.at[slot, pl.ds(j * sub, sub)],
                                  sem_kv.at[a, slot]).start(priority=prio)

        def kv_wait(a, i):
            if nodma: return
            slot = i & (NB - 1)
            dst = (kb, vb)[a].at[slot]
            pltpu.make_async_copy(dst, dst, sem_kv.at[a, slot]).wait()

        def w_start(which, h, r0, nrows, ws=wsub, wp=wpat):
            if nodma: return
            for p in range(nrows // ws):
                rr = _mo(r0 + p * ws, ws)
                if which == 0:
                    src = wq_hbm.at[pl.ds(rr, ws), pl.ds(_mo(h * W, W), W)]
                    dst = wq_v.at[h, pl.ds(rr, ws), :]
                else:
                    src = wo_hbm.at[pl.ds(_mo(h * W + rr, ws), ws), :]
                    dst = wo_v.at[h, pl.ds(rr, ws), :]
                pltpu.make_async_copy(src, dst, sem_w.at[which, h]).start(priority=int(wp[p % len(wp)]))

        def w_wait(which, h):
            if nodma: return
            dst = (wq_v, wo_v)[which].at[h]
            pltpu.make_async_copy(dst, dst, sem_w.at[which, h]).wait()

        def q_piece(u, r):
            h, g = _shr(u, 2), u & 3
            xg = x_v[pl.ds(_mo(g * M, M), M), :]
            w = wq_v[h, :, pl.ds(_mo(r * Dh, Dh), Dh)]
            q = (jnp.dot(xg, w, preferred_element_type=jnp.float32) * qscale).astype(jnp.bfloat16)
            ro = _mo(r * Sq, Sq)
            for bl in range(G):
                q_s[u & 1, bl, pl.ds(ro, Sq), :] = q[bl * Sq:(bl + 1) * Sq, :]

        def o_piece(u, n, width, r0=0, nr=None):
            nr = nr or M
            h, g = _shr(u, 2), u & 3
            cs = pl.ds(_mo(n * width, width), width)
            rs = pl.ds(r0, nr)
            y = jnp.dot(o_s[u & 1, rs, :], wo_v[h, :, cs], preferred_element_type=jnp.float32)
            t = acc[g, rs, cs] + y
            acc[g, rs, cs] = t
            out_v[g, rs, cs] = t.astype(out_v.dtype)

        def out_copy(g, r0, nr, s):
            return pltpu.make_async_copy(out_v.at[g, pl.ds(r0, nr), :],
                                         out_hbm.at[pl.ds(_mo(g * M, M) + r0, nr), :], sem_o.at[s])

        def body(i, c, phase):
            u = _shr(i, 3)
            bl = i & 7
            h, g = _shr(u, 2), u & 3
            slot = i & (NB - 1)
            with sc('kw' + phase):
                kv_wait(0, i)
            vmid = dmid and phase == 'D'
            if not vmid:
                with sc('vw' + phase):
                    kv_wait(1, i)
            if phase == 'B':
                @pl.when(jnp.logical_and(bl == 0, g == 1))
                def _():
                    w_wait(1, h)

                @pl.when(jnp.logical_and(bl == 0, jnp.logical_and(g == 3, h + 1 < Hkv)))
                def _():
                    w_wait(0, h + 1)

            kq = [(0, 0, j) for j in range(nt)]
            vq = [(1, -1, j) for j in range(nt // 2, nt)] + [(1, 0, j) for j in range(nt // 2)]
            pts = [[kq.pop(0) if kvpat[t % len(kvpat)] == 'k' else vq.pop(0)] for t in range(2 * nt)]
            for t in range(2 * nt):
                a_, off_, j_ = pts[t][0]
                assert off_ == -1 or (j_ <= t if a_ == 0 else j_ <= t - nt), (kvpat, t, pts[t])
            if lastsame and phase == 'S':
                pts = [[(0, 0, t)] for t in range(nt)] + [[(1, 0, t)] for t in range(nt)]
                for e in range(nt // 2):
                    pts[e * lastsame // (nt // 2)].insert(e % (nt // 2 // lastsame), (1, -1, nt // 2 + e))
            cnt = [0]

            def wjob():
                hs = W // 2
                pr = hs // G
                if phase == 'A':
                    w_start(1, 0, bl * (W // G), W // G, w0sub_, w0pat_)
                elif phase == 'B':
                    @pl.when(jnp.logical_and(g == 0, h > 0))
                    def _():
                        w_start(1, h, hs + bl * pr, pr)

                    for gg in (1, 2, 3):
                        @pl.when(jnp.logical_and(g == gg, h + 1 < Hkv))
                        def _():
                            w_start(0 if gg < 3 else 1, h + 1, (hs if gg == 2 else 0) + bl * pr, pr)

            def issue(pt):
                if pt == wpos: wjob()
                for (a, off, j) in pts[pt]:
                    prio = int(pat[cnt[0] % len(pat)]); cnt[0] += 1
                    tgt = i + NB + off
                    if phase in ('A', 'B', 'S'):
                        if phase == 'A' and off == -1:
                            @pl.when(i > 0)
                            def _():
                                one(a, tgt, j, prio)
                        else:
                            one(a, tgt, j, prio)
                    elif phase == 'C1':
                        one(a, tgt, j, prio)
                    elif phase == 'C2':
                        if off == -1 and not lastsame:
                            @pl.when(tgt < npair)
                            def _():
                                one(a, tgt, j, prio)

            if nocomp:
                if vmid: kv_wait(1, i)
                for t in range(2 * nt):
                    issue(t)
            else:
                q = q_s[u & 1, bl]
                ss = []
                for t in range(nt):
                    kt = kb[slot, t * sub:(t + 1) * sub, :]
                    ss.append(lax.dot_general(q, kt, NT, preferred_element_type=jnp.float32))
                    issue(t)
                mm = ss[0]
                for t in range(1, nt):
                    mm = jnp.maximum(mm, ss[t])
                m = jnp.max(mm, axis=-1, keepdims=True)
                if phase in ('A', 'B'):
                    q_piece(u + 1, bl)
                if phase == 'B' or (phase in ('C1', 'C2', 'D', 'S') and not msplit):
                    o_piece(u - 1, bl, Dh)
                elif phase in ('C1', 'S'):
                    o_piece(u - 1, bl, 2 * Dh)
                elif phase in ('C2', 'D'):
                    o_piece(u, bl - G // 2, 2 * Dh, 0, M // 2)
                if vmid: kv_wait(1, i)
                o = None
                ll = None
                for t in range(nt):
                    p = jnp.exp2(ss[t] - m)
                    ll = p if ll is None else ll + p
                    pv = jnp.dot(p.astype(jnp.bfloat16), vb[slot, t * sub:(t + 1) * sub, :],
                                 preferred_element_type=jnp.float32)
                    o = pv if o is None else o + pv
                    issue(nt + t)
                l = jnp.sum(ll, axis=-1, keepdims=True)
                inv = pl.reciprocal(l, approx=True)
                inv = inv * (2.0 - l * inv)
                o = (o * inv).astype(jnp.bfloat16)
                ro = _mo(bl * Sq, Sq)
                for r in range(rep):
                    o_s[u & 1, pl.ds(ro, Sq), r * Dh:(r + 1) * Dh] = o[r * Sq:(r + 1) * Sq, :]
            if phase == 'B':
                @pl.when(jnp.logical_and(bl == G - 1, u - 1 >= nunit - ngrp))
                def _():
                    gp = (u - 1) & 3
                    out_copy(gp, 0, M, gp).start()
            elif phase in ('C1', 'S') and msplit:
                @pl.when(bl == G // 2 - 1)
                def _():
                    out_copy(ngrp - 2, 0, M, ngrp - 2).start()
            elif phase == 'D':
                if msplit:
                    out_copy(ngrp - 1, 0, M // 2, ngrp - 1).start()
                else:
                    out_copy(ngrp - 2, 0, M, ngrp - 2).start()
            return c

        if not nodma:
            def pro(i, c):
                @pl.when(i == 0)
                def _():
                    for p in range(B * Sq // xsub):
                        pltpu.make_async_copy(x_hbm.at[pl.ds(p * xsub, xsub), :], x_v.at[pl.ds(p * xsub, xsub), :],
                                              sem_x.at[0]).start(priority=int(xpat[p % len(xpat)]))
                    w_start(0, 0, 0, W, w0sub_, w0pat_)
                return c
            lax.fori_loop(0, 2, pro, 0)

            def pro2(i, c):
                seq = [(a, j * 2 + t) for j in range(nt // 2) for a in range(2) for t in range(2)]
                for cc, (a, j) in enumerate(seq):
                    one(a, i, j, int(ppat[cc % len(ppat)]))
                return c
            lax.fori_loop(0, NB, pro2, 0)
        with sc('zero'):
            acc[...] = jnp.zeros(acc.shape, acc.dtype)
        if not nodma:
            pltpu.make_async_copy(x_v, x_v, sem_x.at[0]).wait()
        w_wait(0, 0)
        if not nocomp:
            def pq(r, c):
                q_piece(0, r)
                return c
            with sc('q0'):
                lax.fori_loop(0, rep, pq, 0)

        n0 = npair - G
        with sc('loopA'):
            lax.fori_loop(0, G, functools.partial(body, phase='A'), 0)
        with sc('loopB'):
            lax.fori_loop(G, n0, functools.partial(body, phase='B'), 0, unroll=unroll)
        if lastsame:
            lax.fori_loop(n0, n0 + G // 2 - 1, functools.partial(body, phase='C1'), 0)
            body(n0 + G // 2 - 1, 0, 'S')
        else:
            with sc('loopC1'):
                lax.fori_loop(n0, n0 + G // 2, functools.partial(body, phase='C1'), 0)
        with sc('loopC2'):
            lax.fori_loop(n0 + G // 2, npair - 1, functools.partial(body, phase='C2'), 0)
        with sc('bodyD'):
            body(npair - 1, 0, 'D')
        r0, nr = (M // 2, M // 2) if msplit else (0, M)
        if not nocomp and not noepi:
            wd = D // osplit
            with sc('epi'):
                for n in range(osplit):
                    o_piece(nunit - 1, n, wd, r0, nr)
        out_copy(ngrp - 1, r0, nr, ngrp).start()
        with sc('outw'):
          for g in range(ngrp - 1):
            out_copy(g, 0, M, g).wait()
          out_copy(ngrp - 1, r0, nr, ngrp).wait()
        if msplit:
            out_copy(ngrp - 1, 0, M // 2, ngrp - 1).wait()

    def fn(x, k_cache, v_cache, wq, wo):
        B, Sq, D = x.shape
        _, Hkv, Sk, Dh = k_cache.shape
        Hq = wq.shape[1] // Dh
        rep = Hq // Hkv
        W = rep * Dh
        kern = functools.partial(kernel, B=B, Hkv=Hkv, rep=rep, Sq=Sq, Dh=Dh, Sk=Sk, D=D)
        bf = jnp.bfloat16
        out = pl.pallas_call(
            kern,
            out_shape=jax.ShapeDtypeStruct((B * Sq, D), x.dtype),
            in_specs=[pl.BlockSpec(memory_space=pl.ANY)] * 5,
            out_specs=pl.BlockSpec(memory_space=pl.ANY),
            scratch_shapes=[
                pltpu.VMEM((NB, Sk, Dh), bf),
                pltpu.VMEM((NB, Sk, Dh), bf),
                pltpu.VMEM((B * Sq, D), bf),
                pltpu.VMEM((Hkv, D, W), bf),
                pltpu.VMEM((Hkv, W, D), bf),
                pltpu.VMEM((2, G, rep * Sq, Dh), bf),
                pltpu.VMEM((2, G * Sq, W), bf),
                pltpu.VMEM((B // G, G * Sq, D), jnp.float32),
                pltpu.VMEM((B // G, G * Sq, D), bf),
                pltpu.SemaphoreType.DMA((2, NB)),
                pltpu.SemaphoreType.DMA((1,)),
                pltpu.SemaphoreType.DMA((2, Hkv)),
                pltpu.SemaphoreType.DMA((B // G + 1,)),
            ],
            compiler_params=pltpu.CompilerParams(vmem_limit_bytes=100 << 20, disable_bounds_checks=nochk, flags=flags, **(extra or {})),
        )(x.reshape(B * Sq, D), k_cache, v_cache, wq, wo)
        return out.reshape(B, Sq, D)
    return fn


_impl = make(**dict(kvpat='kkvv', pat='011', ppat='011', lastsame=1, extra=dict(disable_semaphore_checks=True)))


@jax.jit
def pallas_standalone__gqa_block_cached__sampling_kernel(
    x: jax.Array,
    k_cache: jax.Array,
    v_cache: jax.Array,
    wq: jax.Array,
    wo: jax.Array,
):
    return _impl(x, k_cache, v_cache, wq, wo)
```

```python
import functools

import jax
import jax.numpy as jnp
import numpy as np
from jax import lax
from jax.experimental import pallas as pl
from jax.experimental.pallas import tpu as pltpu

_NT = (((1,), (1,)), ((), ()))
_LOG2E = 1.4426950408889634

G = 8
NB = 4
TILE = 128


def _shr(a, n):
    return a >> n if isinstance(a, int) else lax.shift_right_logical(a, jnp.int32(n))


def _mo(v, m):
    return v if isinstance(v, int) else pl.multiple_of(v, m)


BREV = (0, 8, 4, 12, 2, 10, 6, 14, 1, 9, 5, 13, 3, 11, 7, 15)

SCHED0 = dict(
    pieces={0: [(-1, 0, 256, 0, 128)], 1: [(-1, 256, 256, 0, 128)], 2: [(-1, 512, 256, 0, 128)], 3: [(-1, 768, 256, 0, 128)],
            4: [(0, 0, 512, 0, 64)], 5: [(0, 512, 512, 0, 64)], 6: [], 7: []},
    outs={3: [(-1, 0, 128, 0, 1024)], 5: [(0, 0, 64, 0, 1024)]},
    epi=[(0, 0, 512, 64, 64), (0, 512, 512, 64, 64)],
    vmid=(4, 5, 6, 7),
)


def make(pat='101', kvpat='vvkk', tord=BREV, vord=BREV, ppat='011', wsub=64, w0sub=32, xsub=16, xpat='011', wpos=15,
         sched=SCHED0, nosem=True, nochk=False, nodma=False, nocomp=False, unroll=1, flags=None):

    def kernel(x_hbm, k_hbm, v_hbm, wq_hbm, wo_hbm, out_hbm,
               kb, vb, x_v, wq_v, wo_v, q_s, o_s, acc, out_v, sem_kv, sem_x, sem_w, sem_o,
               *, B, Hkv, rep, Sq, Dh, Sk, D):
        ngrp = B // G
        nunit = Hkv * ngrp
        npair = nunit * G
        W = rep * Dh
        M = G * Sq
        nt = Sk // TILE
        qscale = np.float32((Dh ** -0.5) * _LOG2E)
        assert (rep, W, ngrp, Hkv, B, nt) == (G, D, 4, 4, 32, 16)
        ko, vo = list(tord), list(vord)

        def kv_start(a, i, j, prio):
            if nodma: return
            b, h, slot = i & (B - 1), _shr(i, 5), i & (NB - 1)
            src, dst = ((k_hbm, kb), (v_hbm, vb))[a]
            pltpu.make_async_copy(src.at[b, h, pl.ds(j * TILE, TILE)], dst.at[slot, pl.ds(j * TILE, TILE)],
                                  sem_kv.at[a, slot]).start(priority=prio)

        def kv_wait(a, i):
            if nodma: return
            slot = i & (NB - 1)
            dst = (kb, vb)[a].at[slot]
            pltpu.make_async_copy(dst, dst, sem_kv.at[a, slot]).wait()

        def w_start(which, h, r0, nrows, ws):
            if nodma: return
            for p in range(nrows // ws):
                rr = _mo(r0 + p * ws, ws)
                if which == 0:
                    src = wq_hbm.at[pl.ds(rr, ws), pl.ds(_mo(h * W, W), W)]
                    dst = wq_v.at[h, pl.ds(rr, ws), :]
                else:
                    src = wo_hbm.at[pl.ds(_mo(h * W + rr, ws), ws), :]
                    dst = wo_v.at[h, pl.ds(rr, ws), :]
                pltpu.make_async_copy(src, dst, sem_w.at[which, h]).start()

        def w_wait(which, h):
            if nodma: return
            dst = (wq_v, wo_v)[which].at[h]
            pltpu.make_async_copy(dst, dst, sem_w.at[which, h]).wait()

        def out_copy(g, r0, nr, c0, nc):
            return pltpu.make_async_copy(out_v.at[g, pl.ds(r0, nr), pl.ds(c0, nc)],
                                         out_hbm.at[pl.ds(_mo(g * M, M) + r0, nr), pl.ds(c0, nc)], sem_o.at[0])

        def q_piece(u, r):
            if nocomp: return
            h, g = _shr(u, 2), u & 3
            xg = x_v[pl.ds(_mo(g * M, M), M), :]
            w = wq_v[h, :, pl.ds(_mo(r * Dh, Dh), Dh)]
            q = (jnp.dot(xg, w, preferred_element_type=jnp.float32) * qscale).astype(jnp.bfloat16)
            ro = _mo(r * Sq, Sq)
            for bl in range(G):
                q_s[u & 1, bl, pl.ds(ro, Sq), :] = q[bl * Sq:(bl + 1) * Sq, :]

        def o_piece(u, c0, nc, r0, nr):
            if nocomp: return
            h, g = _shr(u, 2), u & 3
            cs, rs = pl.ds(c0, nc), pl.ds(r0, nr)
            y = jnp.dot(o_s[u & 1, rs, :], wo_v[h, :, cs], preferred_element_type=jnp.float32)
            t = acc[g, rs, cs] + y
            acc[g, rs, cs] = t
            out_v[g, rs, cs] = t.astype(out_v.dtype)

        def pair(i, u, bl, pts, extra, vmid, side):
            slot = i & (NB - 1)
            kv_wait(0, i)
            if not vmid:
                kv_wait(1, i)
            side(-1)

            def issue(t):
                side(t)
                for (a, tgt, j, cond, prio) in pts[t]:
                    if cond is None:
                        kv_start(a, tgt, j, prio)
                    else:
                        pl.when(cond)(functools.partial(kv_start, a, tgt, j, prio))

            if nocomp:
                if vmid: kv_wait(1, i)
                for t in range(2 * nt): issue(t)
                return
            q = q_s[u & 1, bl]
            s = {}
            for t in range(nt):
                kt = kb[slot, ko[t] * TILE:(ko[t] + 1) * TILE, :]
                s[ko[t]] = lax.dot_general(q, kt, _NT, preferred_element_type=jnp.float32)
                issue(t)
            mm = s[ko[0]]
            for t in range(1, nt):
                mm = jnp.maximum(mm, s[ko[t]])
            m = jnp.max(mm, axis=-1, keepdims=True)
            extra()
            if vmid:
                kv_wait(1, i)
            o = ll = None
            for t in range(nt):
                p = jnp.exp2(s[vo[t]] - m)
                ll = p if ll is None else ll + p
                pv = jnp.dot(p.astype(jnp.bfloat16), vb[slot, vo[t] * TILE:(vo[t] + 1) * TILE, :],
                             preferred_element_type=jnp.float32)
                o = pv if o is None else o + pv
                issue(nt + t)
            l = jnp.sum(ll, axis=-1, keepdims=True)
            inv = pl.reciprocal(l, approx=True)
            inv = inv * (2.0 - l * inv)
            o = (o * inv).astype(jnp.bfloat16)
            ro = _mo(bl * Sq, Sq)
            for r in range(rep):
                o_s[u & 1, pl.ds(ro, Sq), r * Dh:(r + 1) * Dh] = o[r * Sq:(r + 1) * Sq, :]

        def refill_points(i, first=False, last=False):
            pts = [[] for _ in range(2 * nt)]
            if last:
                seq = [[(0, i + NB, ko[t], None)] for t in range(nt)] + [[(1, i + NB, vo[t], None)] for t in range(nt)]
                seq[0] = [(1, i + NB - 1, vo[nt // 2 + e], None) for e in range(nt // 2)] + seq[0]
            else:
                kq = [(0, i + NB, ko[j], None, j) for j in range(nt)]
                vq = [(1, i + NB - 1, vo[j], (i > 0) if first else None, -1) for j in range(nt // 2, nt)] + \
                     [(1, i + NB, vo[j], None, nt + j) for j in range(nt // 2)]
                seq = []
                for t in range(2 * nt):
                    e = kq.pop(0) if kvpat[t % len(kvpat)] == 'k' else vq.pop(0)
                    assert e[4] <= t
                    seq.append([e[:4]])
            c = 0
            for t in range(2 * nt):
                for e in seq[t]:
                    pts[t].append(e + (int(pat[c % len(pat)]),))
                    c += 1
            return pts

        def loop_body(i, c, first):
            u, bl = _shr(i, 3), i & (G - 1)
            h, g = _shr(u, 2), u & 3
            hs = W // 2
            pr = hs // G

            def side(t):
                if t == -1 and not first:
                    pl.when(jnp.logical_and(bl == 0, g == 1))(lambda: w_wait(1, h))
                    pl.when(jnp.logical_and(bl == 0, jnp.logical_and(g == 3, h + 1 < Hkv)))(lambda: w_wait(0, h + 1))
                if t == wpos:
                    if first:
                        w_start(1, 0, bl * (W // G), W // G, w0sub)
                    else:
                        pl.when(jnp.logical_and(g == 0, h > 0))(lambda: w_start(1, h, hs + bl * pr, pr, wsub))
                        for gg in (1, 2, 3):
                            pl.when(jnp.logical_and(g == gg, h + 1 < Hkv))(functools.partial(
                                w_start, 0 if gg < 3 else 1, h + 1, (hs if gg == 2 else 0) + bl * pr, pr, wsub))

            def extra():
                q_piece(u + 1, bl)
                if not first:
                    o_piece(u - 1, _mo(bl * Dh, Dh), Dh, 0, M)

            pair(i, u, bl, refill_points(i, first=first), extra, False, side)
            if not first:
                @pl.when(jnp.logical_and(bl == G - 1, u - 1 >= nunit - ngrp))
                def _():
                    out_copy((u - 1) & 3, 0, M, 0, D).start()
            return c

        if not nodma:
            def st_x():
                for p in range(B * Sq // xsub):
                    pltpu.make_async_copy(x_hbm.at[pl.ds(p * xsub, xsub), :], x_v.at[pl.ds(p * xsub, xsub), :],
                                          sem_x.at[0]).start(priority=int(xpat[p % len(xpat)]))

            def st_kv(i):
                seq = [(a, j * 2 + t) for j in range(nt // 2) for a in range(2) for t in range(2)]
                for c, (a, j) in enumerate(seq):
                    kv_start(a, i, j, int(ppat[c % len(ppat)]))

            stages = [st_x, lambda: w_start(0, 0, 0, W, w0sub)] + [functools.partial(st_kv, i) for i in range(NB)]

            def pro(i, c):
                for k_, f_ in enumerate(stages):
                    pl.when(i == k_)(f_)
                return c
            lax.fori_loop(0, len(stages), pro, 0)
        acc[...] = jnp.zeros(acc.shape, acc.dtype)
        if not nodma:
            pltpu.make_async_copy(x_v, x_v, sem_x.at[0]).wait()
        w_wait(0, 0)

        def pq(r, c):
            q_piece(0, r)
            return c
        if not nocomp:
            lax.fori_loop(0, rep, pq, 0)

        n0 = npair - G
        lax.fori_loop(0, G, functools.partial(loop_body, first=True), 0)
        lax.fori_loop(G, n0, functools.partial(loop_body, first=False), 0, unroll=unroll)

        ulast = nunit - 1
        outs = [(g, 0, M, 0, D) for g in range(ngrp - 2)]
        for bl in range(G):
            i = n0 + bl
            if i + NB < npair - 1:
                pts = refill_points(i)
            elif i + NB == npair - 1:
                pts = refill_points(i, last=True)
            else:
                pts = [[] for _ in range(2 * nt)]

            def extra(bl=bl):
                for (du, c0, nc, r0, nr) in sched['pieces'][bl]:
                    o_piece(ulast + du, c0, nc, r0, nr)
            pair(i, ulast, bl, pts, extra, bl in sched['vmid'], lambda t: None)
            for (du, r0, nr, c0, nc) in sched['outs'].get(bl, []):
                outs.append(((ulast + du) & 3, r0, nr, c0, nc))
                out_copy(*outs[-1]).start()
        for (du, c0, nc, r0, nr) in sched['epi']:
            o_piece(ulast + du, c0, nc, r0, nr)
            outs.append(((ulast + du) & 3, r0, nr, c0, nc))
            out_copy(*outs[-1]).start()
        for o_ in outs:
            out_copy(*o_).wait()

    def fn(x, k_cache, v_cache, wq, wo):
        B, Sq, D = x.shape
        _, Hkv, Sk, Dh = k_cache.shape
        rep = wq.shape[1] // Dh // Hkv
        W = rep * Dh
        bf = jnp.bfloat16
        out = pl.pallas_call(
            functools.partial(kernel, B=B, Hkv=Hkv, rep=rep, Sq=Sq, Dh=Dh, Sk=Sk, D=D),
            out_shape=jax.ShapeDtypeStruct((B * Sq, D), x.dtype),
            in_specs=[pl.BlockSpec(memory_space=pl.ANY)] * 5,
            out_specs=pl.BlockSpec(memory_space=pl.ANY),
            scratch_shapes=[
                pltpu.VMEM((NB, Sk, Dh), bf),
                pltpu.VMEM((NB, Sk, Dh), bf),
                pltpu.VMEM((B * Sq, D), bf),
                pltpu.VMEM((Hkv, D, W), bf),
                pltpu.VMEM((Hkv, W, D), bf),
                pltpu.VMEM((2, G, rep * Sq, Dh), bf),
                pltpu.VMEM((2, G * Sq, W), bf),
                pltpu.VMEM((B // G, G * Sq, D), jnp.float32),
                pltpu.VMEM((B // G, G * Sq, D), bf),
                pltpu.SemaphoreType.DMA((2, NB)),
                pltpu.SemaphoreType.DMA((1,)),
                pltpu.SemaphoreType.DMA((2, Hkv)),
                pltpu.SemaphoreType.DMA((1,)),
            ],
            compiler_params=pltpu.CompilerParams(vmem_limit_bytes=64 << 20, disable_bounds_checks=nochk,
                                                 disable_semaphore_checks=nosem, flags=flags),
        )(x.reshape(B * Sq, D), k_cache, v_cache, wq, wo)
        return out.reshape(B, Sq, D)
    return fn


_impl = make()


@jax.jit
def pallas_standalone__gqa_block_cached__sampling_kernel(
    x: jax.Array,
    k_cache: jax.Array,
    v_cache: jax.Array,
    wq: jax.Array,
    wo: jax.Array,
):
    return _impl(x, k_cache, v_cache, wq, wo)
```

```python
import functools

import jax
import jax.numpy as jnp
import numpy as np
from jax import lax
from jax.experimental import pallas as pl
from jax.experimental.pallas import tpu as pltpu

_NT = (((1,), (1,)), ((), ()))
_LOG2E = 1.4426950408889634

_G = 8
_NB = 4
_TILE = 128

_TILE_ORDER = (0, 8, 4, 12, 2, 10, 6, 14, 1, 9, 5, 13, 3, 11, 7, 15)
_STREAM_PATTERN = "vvkk"
_QUEUE_PATTERN = "101"
_PROLOGUE_QUEUES = "011"
_W_ROWS = 64
_W_ROWS_FIRST = 32
_X_ROWS = 16
_W_ISSUE_STEP = 15

_LAST_PIECES = (
    ((-1, 0, 256, 0, 128),), ((-1, 256, 256, 0, 128),), ((-1, 512, 256, 0, 128),), ((-1, 768, 256, 0, 128),),
    ((0, 0, 512, 0, 64),), ((0, 512, 512, 0, 64),), (), (),
)
_LAST_WRITEBACK = {3: (-1, 0, 128), 5: (0, 0, 64)}
_EPILOGUE_PIECES = ((0, 0, 512, 64, 64), (0, 512, 512, 64, 64))
_LATE_V_WAIT = (4, 5, 6, 7)


def _shr(a, n):
    return a >> n if isinstance(a, int) else lax.shift_right_logical(a, jnp.int32(n))


def _mo(v, m):
    return v if isinstance(v, int) else pl.multiple_of(v, m)


def _kernel(x_hbm, k_hbm, v_hbm, wq_hbm, wo_hbm, out_hbm,
            kb, vb, x_v, wq_v, wo_v, q_s, o_s, acc, out_v, sem_kv, sem_x, sem_w, sem_o):
    B, Hkv, Sk, Dh = k_hbm.shape
    D = x_hbm.shape[1]
    W = wq_v.shape[2]
    rep = W // Dh
    M = o_s.shape[1]
    Sq = M // _G
    ngrp = B // _G
    nunit = Hkv * ngrp
    npair = nunit * _G
    nt = Sk // _TILE
    order = _TILE_ORDER
    qscale = np.float32((Dh ** -0.5) * _LOG2E)

    def kv_start(a, i, j, prio):
        b, h, slot = i & (B - 1), _shr(i, 5), i & (_NB - 1)
        src, dst = ((k_hbm, kb), (v_hbm, vb))[a]
        pltpu.make_async_copy(src.at[b, h, pl.ds(j * _TILE, _TILE)], dst.at[slot, pl.ds(j * _TILE, _TILE)],
                              sem_kv.at[a, slot]).start(priority=prio)

    def kv_wait(a, i):
        slot = i & (_NB - 1)
        dst = (kb, vb)[a].at[slot]
        pltpu.make_async_copy(dst, dst, sem_kv.at[a, slot]).wait()

    def w_start(which, h, r0, nrows, step):
        for p in range(nrows // step):
            rr = _mo(r0 + p * step, step)
            if which == 0:
                src = wq_hbm.at[pl.ds(rr, step), pl.ds(_mo(h * W, W), W)]
                dst = wq_v.at[h, pl.ds(rr, step), :]
            else:
                src = wo_hbm.at[pl.ds(_mo(h * W + rr, step), step), :]
                dst = wo_v.at[h, pl.ds(rr, step), :]
            pltpu.make_async_copy(src, dst, sem_w.at[which, h]).start()

    def w_wait(which, h):
        dst = (wq_v, wo_v)[which].at[h]
        pltpu.make_async_copy(dst, dst, sem_w.at[which, h]).wait()

    def out_copy(g, r0, nr, c0, nc):
        return pltpu.make_async_copy(out_v.at[g, pl.ds(r0, nr), pl.ds(c0, nc)],
                                     out_hbm.at[pl.ds(_mo(g * M, M) + r0, nr), pl.ds(c0, nc)], sem_o.at[0])

    def q_piece(u, r):
        h, g = _shr(u, 2), u & 3
        xg = x_v[pl.ds(_mo(g * M, M), M), :]
        w = wq_v[h, :, pl.ds(_mo(r * Dh, Dh), Dh)]
        q = (jnp.dot(xg, w, preferred_element_type=jnp.float32) * qscale).astype(q_s.dtype)
        ro = _mo(r * Sq, Sq)
        for bl in range(_G):
            q_s[u & 1, bl, pl.ds(ro, Sq), :] = q[bl * Sq:(bl + 1) * Sq, :]

    def o_piece(u, c0, nc, r0, nr):
        h, g = _shr(u, 2), u & 3
        cs, rs = pl.ds(c0, nc), pl.ds(r0, nr)
        y = jnp.dot(o_s[u & 1, rs, :], wo_v[h, :, cs], preferred_element_type=jnp.float32)
        t = acc[g, rs, cs] + y
        acc[g, rs, cs] = t
        out_v[g, rs, cs] = t.astype(out_v.dtype)

    def pair(i, u, bl, refill, projections, late_v_wait, side_dma):
        slot = i & (_NB - 1)
        kv_wait(0, i)
        if not late_v_wait:
            kv_wait(1, i)
        side_dma(-1)

        def issue(t):
            side_dma(t)
            for (a, tgt, j, cond, prio) in refill[t]:
                if cond is None:
                    kv_start(a, tgt, j, prio)
                else:
                    pl.when(cond)(functools.partial(kv_start, a, tgt, j, prio))

        q = q_s[u & 1, bl]
        s = []
        for t in range(nt):
            j = order[t]
            kt = kb[slot, j * _TILE:(j + 1) * _TILE, :]
            s.append(lax.dot_general(q, kt, _NT, preferred_element_type=jnp.float32))
            issue(t)
        mm = s[0]
        for t in range(1, nt):
            mm = jnp.maximum(mm, s[t])
        m = jnp.max(mm, axis=-1, keepdims=True)
        projections()
        if late_v_wait:
            kv_wait(1, i)
        o = ll = None
        for t in range(nt):
            j = order[t]
            p = jnp.exp2(s[t] - m)
            ll = p if ll is None else ll + p
            pv = jnp.dot(p.astype(vb.dtype), vb[slot, j * _TILE:(j + 1) * _TILE, :],
                         preferred_element_type=jnp.float32)
            o = pv if o is None else o + pv
            issue(nt + t)
        l = jnp.sum(ll, axis=-1, keepdims=True)
        o = (o / l).astype(o_s.dtype)
        ro = _mo(bl * Sq, Sq)
        for r in range(rep):
            o_s[u & 1, pl.ds(ro, Sq), r * Dh:(r + 1) * Dh] = o[r * Sq:(r + 1) * Sq, :]

    def refill_schedule(i, first_unit=False, final=False):
        if final:
            seq = [[(0, i + _NB, order[t], None)] for t in range(nt)]
            seq += [[(1, i + _NB, order[t], None)] for t in range(nt)]
            seq[0] = [(1, i + _NB - 1, order[e], None) for e in range(nt // 2, nt)] + seq[0]
        else:
            kq = [(0, i + _NB, order[e], None, e) for e in range(nt)]
            vq = [(1, i + _NB - 1, order[e], (i > 0) if first_unit else None, 0) for e in range(nt // 2, nt)]
            vq += [(1, i + _NB, order[e], None, nt + e) for e in range(nt // 2)]
            seq = []
            for t in range(2 * nt):
                e = kq.pop(0) if _STREAM_PATTERN[t % len(_STREAM_PATTERN)] == "k" else vq.pop(0)
                assert e[4] <= t, "a tile may only be refilled after it has been read"
                seq.append([e[:4]])
        out, c = [], 0
        for t in range(2 * nt):
            step = []
            for e in seq[t]:
                step.append(e + (int(_QUEUE_PATTERN[c % len(_QUEUE_PATTERN)]),))
                c += 1
            out.append(step)
        return out

    def loop_body(i, carry, first_unit):
        u, bl = _shr(i, 3), i & (_G - 1)
        h, g = _shr(u, 2), u & 3
        half = W // 2
        rows = half // _G

        def side_dma(t):
            if t == -1 and not first_unit:
                pl.when(jnp.logical_and(bl == 0, g == 1))(lambda: w_wait(1, h))
                pl.when(jnp.logical_and(bl == 0, jnp.logical_and(g == 3, h + 1 < Hkv)))(lambda: w_wait(0, h + 1))
            if t == _W_ISSUE_STEP:
                if first_unit:
                    w_start(1, 0, bl * (W // _G), W // _G, _W_ROWS_FIRST)
                else:
                    pl.when(jnp.logical_and(g == 0, h > 0))(
                        lambda: w_start(1, h, half + bl * rows, rows, _W_ROWS))
                    for gg in (1, 2, 3):
                        pl.when(jnp.logical_and(g == gg, h + 1 < Hkv))(functools.partial(
                            w_start, 0 if gg < 3 else 1, h + 1, (half if gg == 2 else 0) + bl * rows, rows, _W_ROWS))

        def projections():
            q_piece(u + 1, bl)
            if not first_unit:
                o_piece(u - 1, _mo(bl * Dh, Dh), Dh, 0, M)

        pair(i, u, bl, refill_schedule(i, first_unit=first_unit), projections, False, side_dma)
        if not first_unit:
            @pl.when(jnp.logical_and(bl == _G - 1, u - 1 >= nunit - ngrp))
            def _():
                out_copy((u - 1) & 3, 0, M, 0, D).start()
        return carry

    def start_x():
        for p in range(B * Sq // _X_ROWS):
            rs = pl.ds(p * _X_ROWS, _X_ROWS)
            pltpu.make_async_copy(x_hbm.at[rs, :], x_v.at[rs, :], sem_x.at[0]).start(
                priority=int(_PROLOGUE_QUEUES[p % len(_PROLOGUE_QUEUES)]))

    def start_pair(i):
        seq = [(a, j * 2 + e) for j in range(nt // 2) for a in range(2) for e in range(2)]
        for c, (a, j) in enumerate(seq):
            kv_start(a, i, j, int(_PROLOGUE_QUEUES[c % len(_PROLOGUE_QUEUES)]))

    stages = [start_x, lambda: w_start(0, 0, 0, W, _W_ROWS_FIRST)]
    stages += [functools.partial(start_pair, i) for i in range(_NB)]

    def prologue(n, carry):
        for k, stage in enumerate(stages):
            pl.when(n == k)(stage)
        return carry

    lax.fori_loop(0, len(stages), prologue, 0)
    acc[...] = jnp.zeros(acc.shape, acc.dtype)
    pltpu.make_async_copy(x_v, x_v, sem_x.at[0]).wait()
    w_wait(0, 0)

    def first_q(r, carry):
        q_piece(0, r)
        return carry

    lax.fori_loop(0, rep, first_q, 0)

    n0 = npair - _G
    lax.fori_loop(0, _G, functools.partial(loop_body, first_unit=True), 0)
    lax.fori_loop(_G, n0, functools.partial(loop_body, first_unit=False), 0)

    ulast = nunit - 1
    writebacks = [(g, 0, M, 0, D) for g in range(ngrp - 2)]
    for bl in range(_G):
        i = n0 + bl
        if i + _NB < npair - 1:
            refill = refill_schedule(i)
        elif i + _NB == npair - 1:
            refill = refill_schedule(i, final=True)
        else:
            refill = [[] for _ in range(2 * nt)]

        def projections(bl=bl):
            for (du, c0, nc, r0, nr) in _LAST_PIECES[bl]:
                o_piece(ulast + du, c0, nc, r0, nr)

        pair(i, ulast, bl, refill, projections, bl in _LATE_V_WAIT, lambda t: None)
        if bl in _LAST_WRITEBACK:
            du, r0, nr = _LAST_WRITEBACK[bl]
            writebacks.append(((ulast + du) & 3, r0, nr, 0, D))
            out_copy(*writebacks[-1]).start()
    for (du, c0, nc, r0, nr) in _EPILOGUE_PIECES:
        o_piece(ulast + du, c0, nc, r0, nr)
        writebacks.append(((ulast + du) & 3, r0, nr, c0, nc))
        out_copy(*writebacks[-1]).start()
    for wb in writebacks:
        out_copy(*wb).wait()


@jax.jit
def pallas_standalone__gqa_block_cached__sampling_kernel(
    x: jax.Array,
    k_cache: jax.Array,
    v_cache: jax.Array,
    wq: jax.Array,
    wo: jax.Array,
):
    B, Sq, D = x.shape
    _, Hkv, Sk, Dh = k_cache.shape
    W = wq.shape[1] // Hkv
    assert (B, Sq, D, Hkv, Sk, Dh, W) == (32, 16, 1024, 4, 2048, 128, 1024), (x.shape, k_cache.shape, wq.shape)
    assert v_cache.shape == k_cache.shape and wo.shape == (Hkv * W, D)
    dt = k_cache.dtype
    ngrp, M = B // _G, _G * Sq
    out = pl.pallas_call(
        _kernel,
        out_shape=jax.ShapeDtypeStruct((B * Sq, D), x.dtype),
        in_specs=[pl.BlockSpec(memory_space=pl.ANY)] * 5,
        out_specs=pl.BlockSpec(memory_space=pl.ANY),
        scratch_shapes=[
            pltpu.VMEM((_NB, Sk, Dh), dt),
            pltpu.VMEM((_NB, Sk, Dh), v_cache.dtype),
            pltpu.VMEM((B * Sq, D), x.dtype),
            pltpu.VMEM((Hkv, D, W), wq.dtype),
            pltpu.VMEM((Hkv, W, D), wo.dtype),
            pltpu.VMEM((2, _G, W // Dh * Sq, Dh), dt),
            pltpu.VMEM((2, M, W), wo.dtype),
            pltpu.VMEM((ngrp, M, D), jnp.float32),
            pltpu.VMEM((ngrp, M, D), x.dtype),
            pltpu.SemaphoreType.DMA((2, _NB)),
            pltpu.SemaphoreType.DMA((1,)),
            pltpu.SemaphoreType.DMA((2, Hkv)),
            pltpu.SemaphoreType.DMA((1,)),
        ],
        compiler_params=pltpu.CompilerParams(
            vmem_limit_bytes=64 * 1024 * 1024,
            disable_semaphore_checks=True,
        ),
    )(x.reshape(B * Sq, D), k_cache, v_cache, wq, wo)
    return out.reshape(B, Sq, D)
```

```python
import functools

import jax
import jax.numpy as jnp
import numpy as np
from jax import lax
from jax.experimental import pallas as pl
from jax.experimental.pallas import tpu as pltpu

_NT = (((1,), (1,)), ((), ()))
_LOG2E = 1.4426950408889634

_G = 8
_NB = 4
_TILE = 128

_TILE_ORDER = (0, 4, 8, 12, 1, 5, 9, 13, 2, 6, 10, 14, 3, 7, 11, 15)
_STREAM_PATTERN = "vvkk"
_QUEUE_PATTERN = "101"
_PROLOGUE_QUEUES = "011"
_W_ROWS = 64
_W_ROWS_FIRST = 32
_X_ROWS = 16
_W_ISSUE_STEP = 15

_LAST_PIECES = (
    ((-1, 0, 256, 0, 128),), ((-1, 256, 256, 0, 128),), ((-1, 512, 256, 0, 128),), ((-1, 768, 256, 0, 128),),
    ((0, 0, 512, 0, 64),), ((0, 512, 512, 0, 64),), (), (),
)
_LAST_WRITEBACK = {3: (-1, 0, 128), 5: (0, 0, 64)}
_EPILOGUE_PIECES = ((0, 0, 256, 64, 64), (0, 256, 256, 64, 64), (0, 512, 256, 64, 64), (0, 768, 256, 64, 64))


def _shr(a, n):
    return a >> n if isinstance(a, int) else lax.shift_right_logical(a, jnp.int32(n))


def _mo(v, m):
    return v if isinstance(v, int) else pl.multiple_of(v, m)


def _kernel(x_hbm, k_hbm, v_hbm, wq_hbm, wo_hbm, out_hbm,
            kb, vb, x_v, wq_v, wo_v, q_s, o_s, acc, out_v, sem_kv, sem_x, sem_w, sem_o):
    B, Hkv, Sk, Dh = k_hbm.shape
    D = x_hbm.shape[1]
    W = wq_v.shape[2]
    rep = W // Dh
    M = o_s.shape[1]
    Sq = M // _G
    ngrp = B // _G
    nunit = Hkv * ngrp
    npair = nunit * _G
    nt = Sk // _TILE
    order = _TILE_ORDER
    qscale = np.float32((Dh ** -0.5) * _LOG2E)

    def kv_start(a, i, j, prio):
        b, h, slot = i & (B - 1), _shr(i, 5), i & (_NB - 1)
        src, dst = ((k_hbm, kb), (v_hbm, vb))[a]
        pltpu.make_async_copy(src.at[b, h, pl.ds(j * _TILE, _TILE)], dst.at[slot, pl.ds(j * _TILE, _TILE)],
                              sem_kv.at[a, slot]).start(priority=prio)

    def kv_wait(a, i):
        slot = i & (_NB - 1)
        dst = (kb, vb)[a].at[slot]
        pltpu.make_async_copy(dst, dst, sem_kv.at[a, slot]).wait()

    def w_start(which, h, r0, nrows, step):
        for p in range(nrows // step):
            rr = _mo(r0 + p * step, step)
            if which == 0:
                src = wq_hbm.at[pl.ds(rr, step), pl.ds(_mo(h * W, W), W)]
                dst = wq_v.at[h, pl.ds(rr, step), :]
            else:
                src = wo_hbm.at[pl.ds(_mo(h * W + rr, step), step), :]
                dst = wo_v.at[h, pl.ds(rr, step), :]
            pltpu.make_async_copy(src, dst, sem_w.at[which, h]).start()

    def w_wait(which, h):
        dst = (wq_v, wo_v)[which].at[h]
        pltpu.make_async_copy(dst, dst, sem_w.at[which, h]).wait()

    def out_copy(g, r0, nr, c0, nc):
        return pltpu.make_async_copy(out_v.at[g, pl.ds(r0, nr), pl.ds(c0, nc)],
                                     out_hbm.at[pl.ds(_mo(g * M, M) + r0, nr), pl.ds(c0, nc)], sem_o.at[0])

    def q_piece(u, r):
        h, g = _shr(u, 2), u & 3
        xg = x_v[pl.ds(_mo(g * M, M), M), :]
        w = wq_v[h, :, pl.ds(_mo(r * Dh, Dh), Dh)]
        q = (jnp.dot(xg, w, preferred_element_type=jnp.float32) * qscale).astype(q_s.dtype)
        ro = _mo(r * Sq, Sq)
        for bl in range(_G):
            q_s[u & 1, bl, pl.ds(ro, Sq), :] = q[bl * Sq:(bl + 1) * Sq, :]

    def o_piece(u, c0, nc, r0, nr):
        h, g = _shr(u, 2), u & 3
        cs, rs = pl.ds(c0, nc), pl.ds(r0, nr)
        y = jnp.dot(o_s[u & 1, rs, :], wo_v[h, :, cs], preferred_element_type=jnp.float32)
        t = acc[g, rs, cs] + y
        acc[g, rs, cs] = t
        out_v[g, rs, cs] = t.astype(out_v.dtype)

    def pair(i, u, bl, refill, projections, late_v_wait, side_dma):
        slot = i & (_NB - 1)
        kv_wait(0, i)
        if not late_v_wait:
            kv_wait(1, i)
        side_dma(-1)

        def issue(t):
            side_dma(t)
            for (a, tgt, j, cond, prio) in refill[t]:
                if cond is None:
                    kv_start(a, tgt, j, prio)
                else:
                    pl.when(cond)(functools.partial(kv_start, a, tgt, j, prio))

        q = q_s[u & 1, bl]
        s = []
        for t in range(nt):
            j = order[t]
            kt = kb[slot, j * _TILE:(j + 1) * _TILE, :]
            s.append(lax.dot_general(q, kt, _NT, preferred_element_type=jnp.float32))
            issue(t)
        mm = s[0]
        for t in range(1, nt):
            mm = jnp.maximum(mm, s[t])
        m = jnp.max(mm, axis=-1, keepdims=True)
        projections()
        if late_v_wait:
            kv_wait(1, i)
        o = ll = None
        for t in range(nt):
            j = order[t]
            p = jnp.exp2(s[t] - m)
            ll = p if ll is None else ll + p
            pv = jnp.dot(p.astype(vb.dtype), vb[slot, j * _TILE:(j + 1) * _TILE, :],
                         preferred_element_type=jnp.float32)
            o = pv if o is None else o + pv
            issue(nt + t)
        l = jnp.sum(ll, axis=-1, keepdims=True)
        o = (o / l).astype(o_s.dtype)
        ro = _mo(bl * Sq, Sq)
        for r in range(rep):
            o_s[u & 1, pl.ds(ro, Sq), r * Dh:(r + 1) * Dh] = o[r * Sq:(r + 1) * Sq, :]

    def refill_schedule(i, first_unit=False, final=False):
        if final:
            seq = [[(0, i + _NB, order[t], None)] for t in range(nt)]
            seq += [[(1, i + _NB, order[t], None)] for t in range(nt)]
            seq[0] = [(1, i + _NB - 1, order[e], None) for e in range(nt // 2, nt)] + seq[0]
        else:
            kq = [(0, i + _NB, order[e], None, e) for e in range(nt)]
            vq = [(1, i + _NB - 1, order[e], (i > 0) if first_unit else None, 0) for e in range(nt // 2, nt)]
            vq += [(1, i + _NB, order[e], None, nt + e) for e in range(nt // 2)]
            seq = []
            for t in range(2 * nt):
                e = kq.pop(0) if _STREAM_PATTERN[t % len(_STREAM_PATTERN)] == "k" else vq.pop(0)
                assert e[4] <= t, "a tile may only be refilled after it has been read"
                seq.append([e[:4]])
        out, c = [], 0
        for t in range(2 * nt):
            step = []
            for e in seq[t]:
                step.append(e + (int(_QUEUE_PATTERN[c % len(_QUEUE_PATTERN)]),))
                c += 1
            out.append(step)
        return out

    def loop_body(i, carry, first_unit):
        u, bl = _shr(i, 3), i & (_G - 1)
        h, g = _shr(u, 2), u & 3
        half = W // 2
        rows = half // _G

        def side_dma(t):
            if t == -1 and not first_unit:
                pl.when(jnp.logical_and(bl == 0, g == 1))(lambda: w_wait(1, h))
                pl.when(jnp.logical_and(bl == 0, jnp.logical_and(g == 3, h + 1 < Hkv)))(lambda: w_wait(0, h + 1))
            if t == _W_ISSUE_STEP:
                if first_unit:
                    w_start(1, 0, bl * (W // _G), W // _G, _W_ROWS_FIRST)
                else:
                    pl.when(jnp.logical_and(g == 0, h > 0))(
                        lambda: w_start(1, h, half + bl * rows, rows, _W_ROWS))
                    for gg in (1, 2, 3):
                        pl.when(jnp.logical_and(g == gg, h + 1 < Hkv))(functools.partial(
                            w_start, 0 if gg < 3 else 1, h + 1, (half if gg == 2 else 0) + bl * rows, rows, _W_ROWS))

        def projections():
            q_piece(u + 1, bl)
            if not first_unit:
                o_piece(u - 1, _mo(bl * Dh, Dh), Dh, 0, M)

        pair(i, u, bl, refill_schedule(i, first_unit=first_unit), projections, False, side_dma)
        if not first_unit:
            @pl.when(jnp.logical_and(bl == _G - 1, u - 1 >= nunit - ngrp))
            def _():
                out_copy((u - 1) & 3, 0, M, 0, D).start()
        return carry

    def start_x():
        for p in range(B * Sq // _X_ROWS):
            rs = pl.ds(p * _X_ROWS, _X_ROWS)
            pltpu.make_async_copy(x_hbm.at[rs, :], x_v.at[rs, :], sem_x.at[0]).start(
                priority=int(_PROLOGUE_QUEUES[p % len(_PROLOGUE_QUEUES)]))

    def start_pair(i):
        seq = [(a, j * 2 + e) for j in range(nt // 2) for a in range(2) for e in range(2)]
        for c, (a, j) in enumerate(seq):
            kv_start(a, i, j, int(_PROLOGUE_QUEUES[c % len(_PROLOGUE_QUEUES)]))

    stages = [start_x, lambda: w_start(0, 0, 0, W, _W_ROWS_FIRST)]
    stages += [functools.partial(start_pair, i) for i in range(_NB)]

    def prologue(n, carry):
        for k, stage in enumerate(stages):
            pl.when(n == k)(stage)
        return carry

    lax.fori_loop(0, len(stages), prologue, 0)
    acc[...] = jnp.zeros(acc.shape, acc.dtype)
    pltpu.make_async_copy(x_v, x_v, sem_x.at[0]).wait()
    w_wait(0, 0)

    def first_q(r, carry):
        q_piece(0, r)
        return carry

    lax.fori_loop(0, rep, first_q, 0)

    n0 = npair - _G
    lax.fori_loop(0, _G, functools.partial(loop_body, first_unit=True), 0)
    lax.fori_loop(_G, n0, functools.partial(loop_body, first_unit=False), 0)

    ulast = nunit - 1
    writebacks = [(g, 0, M, 0, D) for g in range(ngrp - 2)]
    for bl in range(_G):
        i = n0 + bl
        if i + _NB < npair - 1:
            refill = refill_schedule(i)
        elif i + _NB == npair - 1:
            refill = refill_schedule(i, final=True)
        else:
            refill = [[] for _ in range(2 * nt)]

        def projections(bl=bl):
            for (du, c0, nc, r0, nr) in _LAST_PIECES[bl]:
                o_piece(ulast + du, c0, nc, r0, nr)

        pair(i, ulast, bl, refill, projections, True, lambda t: None)
        if bl in _LAST_WRITEBACK:
            du, r0, nr = _LAST_WRITEBACK[bl]
            writebacks.append(((ulast + du) & 3, r0, nr, 0, D))
            out_copy(*writebacks[-1]).start()
    for (du, c0, nc, r0, nr) in _EPILOGUE_PIECES:
        o_piece(ulast + du, c0, nc, r0, nr)
        writebacks.append(((ulast + du) & 3, r0, nr, c0, nc))
        out_copy(*writebacks[-1]).start()
    for wb in writebacks:
        out_copy(*wb).wait()


@jax.jit
def pallas_standalone__gqa_block_cached__sampling_kernel(
    x: jax.Array,
    k_cache: jax.Array,
    v_cache: jax.Array,
    wq: jax.Array,
    wo: jax.Array,
):
    B, Sq, D = x.shape
    _, Hkv, Sk, Dh = k_cache.shape
    W = wq.shape[1] // Hkv
    assert (B, Sq, D, Hkv, Sk, Dh, W) == (32, 16, 1024, 4, 2048, 128, 1024), (x.shape, k_cache.shape, wq.shape)
    assert v_cache.shape == k_cache.shape and wo.shape == (Hkv * W, D)
    dt = k_cache.dtype
    ngrp, M = B // _G, _G * Sq
    out = pl.pallas_call(
        _kernel,
        out_shape=jax.ShapeDtypeStruct((B * Sq, D), x.dtype),
        in_specs=[pl.BlockSpec(memory_space=pl.ANY)] * 5,
        out_specs=pl.BlockSpec(memory_space=pl.ANY),
        scratch_shapes=[
            pltpu.VMEM((_NB, Sk, Dh), dt),
            pltpu.VMEM((_NB, Sk, Dh), v_cache.dtype),
            pltpu.VMEM((B * Sq, D), x.dtype),
            pltpu.VMEM((Hkv, D, W), wq.dtype),
            pltpu.VMEM((Hkv, W, D), wo.dtype),
            pltpu.VMEM((2, _G, W // Dh * Sq, Dh), dt),
            pltpu.VMEM((2, M, W), wo.dtype),
            pltpu.VMEM((ngrp, M, D), jnp.float32),
            pltpu.VMEM((ngrp, M, D), x.dtype),
            pltpu.SemaphoreType.DMA((2, _NB)),
            pltpu.SemaphoreType.DMA((1,)),
            pltpu.SemaphoreType.DMA((2, Hkv)),
            pltpu.SemaphoreType.DMA((1,)),
        ],
        compiler_params=pltpu.CompilerParams(
            vmem_limit_bytes=64 * 1024 * 1024,
            disable_semaphore_checks=True,
        ),
    )(x.reshape(B * Sq, D), k_cache, v_cache, wq, wo)
    return out.reshape(B, Sq, D)
```
